```python
import jax
import jax.numpy as jnp

def _softmax(x, axis=-1):
    return jax.nn.softmax(x, axis=axis)
def _gelu(x):
    return jax.nn.gelu(x, approximate=True)
def _silu(x):
    return jax.nn.silu(x)
def _sigmoid(x):
    return jax.nn.sigmoid(x)
def _layernorm(x, axis=-1, eps=1e-5):
    m = jnp.mean(x, axis=axis, keepdims=True)
    v = jnp.var(x, axis=axis, keepdims=True)
    return (x - m) / jnp.sqrt(v + eps)
def _scatter_add(tgt, idx, src, axis=0):
    return tgt.at[idx].add(src)
def _segment_sum(src, seg, n):
    return jax.ops.segment_sum(src, seg, n)
class _Rng:
    def __init__(self, key):
        self._k = key
    def _next(self):
        self._k, sub = jax.random.split(self._k)
        return sub
    def normal(self, shape):
        return jax.random.normal(self._next(), shape, dtype=jnp.bfloat16)
    def randint(self, lo, hi, shape):
        return jax.random.randint(self._next(), shape, lo, hi, dtype=jnp.int32)
    def uniform(self, shape, lo=0.0, hi=1.0):
        return jax.random.uniform(self._next(), shape, jnp.bfloat16, lo, hi)
    def permutation(self, n):
        return jax.random.permutation(self._next(), n)


kernel_name = 'recurrent_scan__sliding_block_cached__moe_arch_mod__decode'

def setup_inputs():
    _rng = _Rng(jax.random.key(int.from_bytes(__import__("os").urandom(4), "little")))
    _w = (lambda a: (lambda t: t.astype(jnp.bfloat16) if jnp.issubdtype(t.dtype, jnp.floating) else t)(jnp.asarray(a)))
    def _A_setup():
        B, Sq, D = 1, 1, 512
        Hq, Hkv, Sk, Dh = 32, 32, 32768, 128
        assert Hq % Hkv == 0, (Hq, Hkv)
        return {
            "x": _w((lambda *s: _rng.normal(s) * 0.05)(B, Sq, D)),
            "k_cache": _w((lambda *s: _rng.normal(s) * 0.05)(B, Hkv, Sk, Dh)),
            "v_cache": _w((lambda *s: _rng.normal(s) * 0.05)(B, Hkv, Sk, Dh)),
            "wq": _w((lambda *s: _rng.normal(s) * 0.05)(D, Hq * Dh) * (D ** -0.5)),
            "wo": _w((lambda *s: _rng.normal(s) * 0.05)(Hq * Dh, D) * ((Hq * Dh) ** -0.5)),
        }
    _A_in = _A_setup()

    def _B_setup():
        B, S, D, F, C = 1, 1, 512, 1376, 1
        return {
            "x": _w((lambda *s: _rng.normal(s) * 0.05)(B, S, D)),
            "w_r": _w((lambda *s: _rng.normal(s) * 0.05)(D)),
            "w_gate": _w((lambda *s: _rng.normal(s) * 0.05)(D, F)),
            "w_up": _w((lambda *s: _rng.normal(s) * 0.05)(D, F)),
            "w_down": _w((lambda *s: _rng.normal(s) * 0.05)(F, D)),
        }
    _B_in = _B_setup()

    return {
        "A_x": _A_in["x"],
        "A_k_cache": _A_in["k_cache"],
        "A_v_cache": _A_in["v_cache"],
        "A_wq": _A_in["wq"],
        "A_wo": _A_in["wo"],
        "B_x": _B_in["x"],
        "B_w_r": _B_in["w_r"],
        "B_w_gate": _B_in["w_gate"],
        "B_w_up": _B_in["w_up"],
        "B_w_down": _B_in["w_down"],
    }

def reference(A_x, A_k_cache, A_v_cache, A_wq, A_wo, B_x, B_w_r, B_w_gate, B_w_up, B_w_down):
    def _A_ref(x, k_cache, v_cache, wq, wo):
        B, Sq, D = x.shape
        Hq, Dh = 32, 128
        Hkv, Sk = k_cache.shape[1], k_cache.shape[2]
        W = min(4096, max(256, Sk // 4))
        rep = Hq // Hkv
        q = (lambda x, *d: x.transpose(*d))((x @ wq).reshape(B, Sq, Hq, Dh), 0, 2, 1, 3)
        k = jnp.repeat(k_cache[:, :, Sk - W:, :], rep, axis=1)
        v = jnp.repeat(v_cache[:, :, Sk - W:, :], rep, axis=1)
        scores = jnp.einsum("bhqd,bhkd->bhqk", q, k) * (Dh ** -0.5)
        p = _softmax(scores, axis=-1)
        o = jnp.einsum("bhqk,bhkd->bhqd", p, v)
        return (lambda x, *d: x.transpose(*d))(o, 0, 2, 1, 3).reshape(B, Sq, Hq * Dh) @ wo

    def _B_ref(x, w_r, w_gate, w_up, w_down):
        B, S, D = x.shape
        C = 1
        r = x @ w_r
        idx = jnp.argsort(-r, axis=-1)[:, :C]
        idx_e = jnp.repeat(idx.reshape(B, C, 1), D, axis=2)
        x_sel = jnp.take_along_axis(x, idx_e, axis=1)
        g = _silu(x_sel @ w_gate)
        u = x_sel @ w_up
        y = (g * u) @ w_down
        r_sel = _sigmoid(jnp.take_along_axis(r, idx, axis=1))
        y = y * r_sel.reshape(B, C, 1)
        b_off = (jnp.arange(B) * S).reshape(B, 1)
        flat_idx = (idx + b_off).reshape(B * C)
        zero = (x * 0.0).reshape(B * S, D)
        upd = _scatter_add(zero, flat_idx, y.reshape(B * C, D), axis=0)
        return x + upd.reshape(B, S, D)

    x = A_x
    xn = _layernorm(x, axis=-1)
    s = _A_ref(xn, A_k_cache, A_v_cache, A_wq, A_wo)
    g = _silu(_B_ref(xn, B_w_r, B_w_gate, B_w_up, B_w_down))
    return x + s * g
```

```python
import jax
import jax.numpy as jnp
import jax.experimental.pallas as pl
import jax.experimental.pallas.tpu as pltpu

D = 512
NH = 32
DH = 128
SK = 32768
W = min(4096, max(256, SK // 4))
F = 1376

G = 8
NG = NH // G
PR = 64
NR = W // PR
WR = 16
OB = NH * DH // 8
NB = (OB - DH) // WR
TA = DH // WR
VS = (8, 24, 16, 12, 4)
LAG = 2 * VS[0] + NB - TA
PRE = 25
QK0 = 10
TAIL = (16, 8, 4, 1, 1, 1, 1)

BF16 = jnp.bfloat16
F32 = jnp.float32
_NT = (((1,), (1,)), ((), ()))
LOW, HIGH = 1, 0


def _times(i, n):
    return i * n if isinstance(i, int) else pl.multiple_of(i * n, n)


def _head(g, hh):
    return (g % 2) * 4 + (g // 2) * 16 + hh % 4 + (hh // 4) * 8


def _wait_all(dst, sem):
    pltpu.make_async_copy(dst, dst, sem).wait()


def _kernel(x_h, k_h, v_h, wq_h, wo_h, wr_h, wg_h, wu_h, wd_h, out_ref,
            x_v, wr_v, wq_v, kv_v, wo_v, wf_v, q_v, o_v, p_v, l_v, c_v,
            s_x, s_w, s_kv, s_v, s_wo, s_t):
    kv_h = (k_h, v_h)
    wf_h = (wg_h, wu_h, wd_h)

    def kv(t, n, u, sem=None):
        g, j = n // NR, n % NR
        return pltpu.make_async_copy(
            kv_h[t].at[0, pl.ds(_head(g, 2 * u), 2), pl.ds(_times((SK - W) // PR + j, PR), PR), :],
            kv_v.at[t, g, pl.ds(2 * u, 2), pl.ds(_times(j, PR), PR), :],
            s_kv.at[t, g % 2] if sem is None else sem)

    def wq(i):
        idx = (slice(None), pl.ds(i % 4 * 64 + i // 16 * 8, 8), pl.ds(i // 4 % 4 * 1024, 1024))
        return pltpu.make_async_copy(wq_h.at[idx], wq_v.at[idx], s_w.at[0])

    def wf(i):
        rows = pl.ds(i // 3 * WR, WR)
        return pltpu.make_async_copy(wf_h[i % 3].at[:, rows, :], wf_v.at[i % 3, :, rows, :], s_w.at[1])

    def wo(m, u, sem):
        rows = pl.ds(_times(m, WR), WR)
        return pltpu.make_async_copy(wo_h.at[:, u, rows, :], wo_v.at[:, u, rows, :], sem)

    def send(n0, cnt, low=lambda n, u: kv(1, n - LAG, u), high=lambda n, u: kv(0, n, u)):
        def body(i, c):
            for u in range(4):
                low(n0 + i, u).start(priority=LOW)
                high(n0 + i, u).start(priority=HIGH)
            return c
        if cnt:
            jax.lax.fori_loop(0, cnt, body, 0)

    def per_head(work, n0, cnt, *pieces):
        def body(hh, c):
            work(hh)
            send(n0 + hh * cnt, cnt, *pieces)
            return c
        jax.lax.fori_loop(0, G, body, 0)

    copy_x = pltpu.make_async_copy(x_h, x_v, s_x.at[0])
    copy_wr = pltpu.make_async_copy(wr_h, wr_v, s_x.at[1])
    first = ([wf(i) for i in range(3 * F // (2 * WR))] + [wq(i) for i in range(128)]
             + [kv(0, n, u) for n in range(LAG) for u in range(4)])
    n_low = (len(first) + PRE) // 2
    assert 2 * n_low - PRE == len(first)
    for i in range(n_low):
        if i == 8:
            copy_x.start()
            copy_wr.start()
        first[i].start(priority=LOW)
        if i >= PRE:
            first[n_low + i - PRE].start(priority=HIGH)
    copy_x.wait()
    copy_wr.wait()

    x = x_v[0].astype(F32)
    mean = jnp.mean(x, axis=-1, keepdims=True)
    var = jnp.mean(jnp.square(x - mean), axis=-1, keepdims=True)
    xn_b = ((x - mean) / jnp.sqrt(var + 1e-5)).astype(BF16)
    xn = xn_b.astype(F32)
    x8 = jnp.broadcast_to(x, (8, D))
    xn8 = jnp.broadcast_to(xn_b, (8, D))
    r = jnp.sum(xn * wr_v[...].reshape(1, D).astype(F32), axis=-1, keepdims=True)
    send(LAG, 16)

    _wait_all(wf_v, s_w.at[1])

    def ffn(k, y):
        gt = jax.lax.dot_general(xn8, wf_v[0, k], _NT, preferred_element_type=F32)
        up = jax.lax.dot_general(xn8, wf_v[1, k], _NT, preferred_element_type=F32)
        hid = (jax.nn.silu(gt) * up).astype(BF16)
        y = y + jnp.dot(hid, wf_v[2, k], preferred_element_type=F32)
        send(LAG + 16 + 4 * k, 4)
        return y
    y = jax.lax.fori_loop(0, 2, ffn, jnp.zeros((8, D), F32))
    upd = xn * 0.0 + y * jax.nn.sigmoid(r)
    gate = jax.nn.silu(xn + upd)

    _wait_all(wq_v, s_w.at[0])

    def project(c):
        cols = pl.ds(_times(c, 4 * DH), 4 * DH)
        q = (jnp.dot(xn8[:, :D // 2], wq_v[0, :, cols], preferred_element_type=F32)
             + jnp.dot(xn8[:, D // 2:], wq_v[1, :, cols], preferred_element_type=F32))
        for t in range(4):
            q_v[c * 4 + t] = q[:, t * DH:(t + 1) * DH]
    per_head(project, LAG + 24, 1)
    send(LAG + 24 + G, NR - LAG - 24 - G)

    def probs(g, hh):
        s = jax.lax.dot_general(q_v[_head(g, hh)].astype(BF16), kv_v[0, g, hh], _NT,
                                preferred_element_type=F32) * DH ** -0.5
        p = jnp.exp(s - jnp.max(s, axis=-1, keepdims=True))
        p_v[hh] = p
        l_v[hh] = jnp.broadcast_to(jnp.sum(p, axis=-1, keepdims=True), (8, DH))

    def attend(g, hh):
        o = jnp.dot(p_v[hh].astype(BF16), kv_v[1, g, hh], preferred_element_type=F32)
        o_v[_head(g, hh)] = o / l_v[hh]

    edges = [sum(VS[:c]) for c in range(len(VS) + 1)]

    def v_last(n, u):
        j = n - LAG + VS[0] - (NG - 1) * NR
        return kv(1, n - LAG + VS[0], u, s_v.at[sum(jnp.where(j >= e, 1, 0) for e in edges[1:-1])])

    def group(g, c):
        n0 = (g + 1) * NR
        send(n0, QK0)
        _wait_all(kv_v.at[0, g], s_kv.at[0, g % 2])
        per_head(lambda hh: probs(g, hh), n0 + QK0, 2)
        send(n0 + QK0 + 2 * G, LAG - QK0 - 2 * G)

        def rest(*pieces):
            send(n0 + LAG, NR - 2 * G - LAG, *pieces)
            _wait_all(kv_v.at[1, g], s_kv.at[1, g % 2])
            per_head(lambda hh: attend(g, hh), n0 + NR - 2 * G, 2, *pieces)
        pl.when(g < NG - 2)(rest)
        pl.when(g == NG - 2)(lambda: rest(v_last))
        return c
    jax.lax.fori_loop(0, NG - 1, group, 0)

    g = NG - 1
    n0 = NG * NR + VS[0]
    CH = DH // WR
    tail_edges = [sum(TAIL[:c]) for c in range(1, len(TAIL))]

    def wo_main(n, u):
        return wo(n - n0, u, s_wo.at[(n - n0) // CH])

    def wo_tail(n, u):
        m = n - n0 - (NB - TA)
        return wo(NB + m, u, s_t.at[sum(jnp.where(4 * m + u >= e, 1, 0) for e in tail_edges)])

    def attend_slice(c):
        rows = pl.ds(edges[c] * PR, VS[c] * PR)
        _wait_all(kv_v.at[1, g, :, rows], s_v.at[c])

        def work(hh):
            o = jnp.dot(p_v[hh, :, rows].astype(BF16), kv_v[1, g, hh, rows], preferred_element_type=F32)
            if c > 0:
                o = o + o_v[_head(g, hh)]
            o_v[_head(g, hh)] = o / l_v[hh] if c == len(VS) - 1 else o
        return work

    def project_out(acc, r0, r1, heads):
        for h in heads:
            lo, hi = max(r0, h % 4 * DH), min(r1, (h % 4 + 1) * DH)
            if lo < hi:
                acc = acc + jnp.dot(o_v[h].astype(BF16)[:, lo % DH:lo % DH + hi - lo],
                                    wo_v[h // 16, h // 4 % 4, pl.ds(lo, hi - lo), :], preferred_element_type=F32)
        return acc

    def columns(heads):
        for h in heads:
            if h % 4 == 3:
                o = o_v[h].astype(BF16).astype(F32)
                c_v[h // 4] = jnp.broadcast_to(o[0:1], (DH, DH)).T

    def wait_wo(c):
        _wait_all(wo_v.at[:, :, pl.ds(c * DH, DH), :], s_wo.at[c])

    assert (NB - TA) % G == 0 and TA % G == 0 and sum(TAIL) == 4 * TA and sum(VS) == NR
    send(NG * NR, VS[0], v_last, lambda n, u: kv(1, n - NR, u, s_v.at[0]))
    _wait_all(kv_v.at[0, g], s_kv.at[0, g % 2])
    per_head(lambda hh: probs(g, hh), n0, (NB - TA) // G, v_last, wo_main)
    slice0, slice1 = attend_slice(0), attend_slice(1)
    per_head(lambda hh: (slice0(hh), slice1(hh)), n0 + NB - TA, TA // G, wo_tail, wo_main)

    last = [_head(g, hh) for hh in range(G)]
    early = [h for h in range(NH) if h not in last]
    acc = jnp.zeros((8, D), F32)
    columns(early)
    for c in range(2, len(VS)):
        if c - 2 < NB // CH - 1:
            wait_wo(c - 2)
            acc = project_out(acc, (c - 2) * DH, (c - 1) * DH, early)
        work = attend_slice(c)
        for hh in range(G):
            work(hh)
    columns(last)
    acc = project_out(acc, 0, NB * WR - DH, last)
    wait_wo(NB // CH - 1)
    acc = project_out(acc, NB * WR - DH, NB * WR, range(NH))

    part = jnp.zeros((8, D), F32)
    row = jax.lax.broadcasted_iota(jnp.int32, (8, D), 0)
    i0 = 0
    for c, n in enumerate(TAIL):
        r0 = (NB + i0 // 4) * WR
        blocks = slice(None) if n % 4 == 0 else pl.ds(i0 % 4, n)
        _wait_all(wo_v.at[:, blocks, pl.ds(r0, pl.cdiv(n, 4) * WR), :], s_t.at[c])
        if c == 0:
            acc = project_out(acc, r0, r0 + n // 4 * WR, range(NH))
        else:
            for i in range(i0, i0 + n):
                for k in range(2):
                    coef = c_v[4 * k + i % 4, pl.ds(i // 4 * WR, WR), :]
                    t = (wo_v[k, i % 4, pl.ds((NB + i // 4) * WR, WR), :].astype(F32)
                         * jnp.concatenate([coef] * (D // DH), axis=1))
                    part = part + (t[:8] + t[8:])
        if c == 2:
            part = part + jnp.where(row == 0, acc, 0.0)
        i0 += n
    s_out = jnp.sum(part, axis=0, keepdims=True)

    res = x8 + jnp.broadcast_to(s_out, (8, D)) * gate
    out_ref[0] = res.astype(out_ref.dtype)[0:1]


@jax.jit
def pallas_recurrent_scan__sliding_block_cached__moe_arch_mod__decode_kernel(
    A_x: jax.Array,
    A_k_cache: jax.Array,
    A_v_cache: jax.Array,
    A_wq: jax.Array,
    A_wo: jax.Array,
    B_x: jax.Array,
    B_w_r: jax.Array,
    B_w_gate: jax.Array,
    B_w_up: jax.Array,
    B_w_down: jax.Array,
):
    del B_x
    hbm = pl.BlockSpec(memory_space=pltpu.HBM)
    dma = pltpu.SemaphoreType.DMA
    halves = (2, F // 2, D)
    return pl.pallas_call(
        _kernel,
        out_shape=jax.ShapeDtypeStruct((1, 1, D), BF16),
        in_specs=[hbm] * 9,
        out_specs=pl.BlockSpec(memory_space=pltpu.VMEM),
        scratch_shapes=[
            pltpu.VMEM((1, 1, D), BF16),
            pltpu.VMEM((D,), BF16),
            pltpu.VMEM((2, D // 2, NH * DH), BF16),
            pltpu.VMEM((2, NG, G, W, DH), BF16),
            pltpu.VMEM((2, 4, OB, D), BF16),
            pltpu.VMEM((3,) + halves, BF16),
            pltpu.VMEM((NH, 8, DH), F32),
            pltpu.VMEM((NH, 8, DH), F32),
            pltpu.VMEM((G, 8, W), F32),
            pltpu.VMEM((G, 8, DH), F32),
            pltpu.VMEM((8, DH, DH), F32),
            dma((2,)), dma((2,)), dma((2, 2)), dma((len(VS),)), dma((NB * WR // DH,)), dma((len(TAIL),)),
        ],
        compiler_params=pltpu.CompilerParams(
            vmem_limit_bytes=100 * 1024 * 1024,
            disable_semaphore_checks=True,
        ),
    )(A_x, A_k_cache, A_v_cache, A_wq.reshape(2, D // 2, NH * DH), A_wo.reshape(2, 4, OB, D), B_w_r,
      B_w_gate.T.reshape(halves), B_w_up.T.reshape(halves), B_w_down.reshape(halves))
```

```python
import jax
import jax.numpy as jnp
import jax.experimental.pallas as pl
import jax.experimental.pallas.tpu as pltpu

D = 512
NH = 32
DH = 128
SK = 32768
W = min(4096, max(256, SK // 4))
F = 1376

G = 8
NG = NH // G
PR = 64
NR = W // PR
WR = 16
OB = NH * DH // 8
NB = (OB - DH) // WR
TA = DH // WR
VS = (8, 24, 16, 12, 4)
LAG = 2 * VS[0] + NB - TA
PRE = 25
QK0 = 10
TAIL = (16, 8, 4, 1, 1, 1, 1)

BF16 = jnp.bfloat16
F32 = jnp.float32
_NT = (((1,), (1,)), ((), ()))
LOW, HIGH = 1, 0


def _times(i, n):
    return i * n if isinstance(i, int) else pl.multiple_of(i * n, n)


def _wait_all(dst, sem):
    pltpu.make_async_copy(dst, dst, sem).wait()


def _kernel(x_h, k_h, v_h, wq_h, wo_h, wr_h, wg_h, wu_h, wd_h, out_ref,
            x_v, wr_v, wq_v, kv_v, wo_v, wf_v, q_v, o_v, p_v, l_v, c_v,
            s_x, s_w, s_kv, s_v, s_wo, s_t):
    kv_h = (k_h, v_h)
    wf_h = (wg_h, wu_h, wd_h)

    def kv(t, n, u, sem=None):
        g, j = n // NR, n % NR
        return pltpu.make_async_copy(
            kv_h[t].at[0, pl.ds(g * G + 2 * u, 2), pl.ds(_times((SK - W) // PR + j, PR), PR), :],
            kv_v.at[t, g, pl.ds(2 * u, 2), pl.ds(_times(j, PR), PR), :],
            s_kv.at[t, g % 2] if sem is None else sem)

    def wq(i):
        idx = (slice(None), pl.ds(i % 4 * 64 + i // 16 * 8, 8), pl.ds(i // 4 % 4 * 1024, 1024))
        return pltpu.make_async_copy(wq_h.at[idx], wq_v.at[idx], s_w.at[0])

    def wf(i):
        rows = pl.ds(i // 3 * WR, WR)
        return pltpu.make_async_copy(wf_h[i % 3].at[:, rows, :], wf_v.at[i % 3, :, rows, :], s_w.at[1])

    def wo(m, u, sem):
        rows = pl.ds(_times(m, WR), WR)
        return pltpu.make_async_copy(wo_h.at[:, u, rows, :], wo_v.at[:, u, rows, :], sem)

    def send(n0, cnt, low=lambda n, u: kv(1, n - LAG, u), high=lambda n, u: kv(0, n, u)):
        def body(i, c):
            for u in range(4):
                high(n0 + i, u).start(priority=HIGH)
                low(n0 + i, u).start(priority=LOW)
            return c
        if cnt:
            jax.lax.fori_loop(0, cnt, body, 0)

    def per_head(work, n0, cnt, *pieces):
        def body(hh, c):
            work(hh)
            send(n0 + hh * cnt, cnt, *pieces)
            return c
        jax.lax.fori_loop(0, G, body, 0)

    copy_x = pltpu.make_async_copy(x_h, x_v, s_x.at[0])
    copy_wr = pltpu.make_async_copy(wr_h, wr_v, s_x.at[1])
    first = ([wf(i) for i in range(3 * F // (2 * WR))] + [wq(i) for i in range(128)]
             + [kv(0, n, u) for n in range(LAG) for u in range(4)])
    n_low = (len(first) + PRE) // 2
    assert 2 * n_low - PRE == len(first)
    for i in range(n_low):
        if i == PRE:
            copy_x.start()
            copy_wr.start()
        first[i].start(priority=LOW)
        if i >= PRE:
            first[n_low + i - PRE].start(priority=HIGH)
    copy_x.wait()
    copy_wr.wait()

    x = x_v[0].astype(F32)
    mean = jnp.mean(x, axis=-1, keepdims=True)
    var = jnp.mean(jnp.square(x - mean), axis=-1, keepdims=True)
    xn_b = ((x - mean) / jnp.sqrt(var + 1e-5)).astype(BF16)
    xn = xn_b.astype(F32)
    x8 = jnp.broadcast_to(x, (8, D))
    xn8 = jnp.broadcast_to(xn_b, (8, D))
    r = jnp.sum(xn * wr_v[...].reshape(1, D).astype(F32), axis=-1, keepdims=True)
    send(LAG, 16)

    _wait_all(wf_v, s_w.at[1])

    def ffn(k, y):
        gt = jax.lax.dot_general(xn8, wf_v[0, k], _NT, preferred_element_type=F32)
        up = jax.lax.dot_general(xn8, wf_v[1, k], _NT, preferred_element_type=F32)
        hid = (jax.nn.silu(gt) * up).astype(BF16)
        y = y + jnp.dot(hid, wf_v[2, k], preferred_element_type=F32)
        send(LAG + 16 + 4 * k, 4)
        return y
    y = jax.lax.fori_loop(0, 2, ffn, jnp.zeros((8, D), F32))
    upd = xn * 0.0 + y * jax.nn.sigmoid(r)
    gate = jax.nn.silu(xn + upd)

    _wait_all(wq_v, s_w.at[0])

    def project(c):
        cols = pl.ds(_times(c, 4 * DH), 4 * DH)
        q = (jnp.dot(xn8[:, :D // 2], wq_v[0, :, cols], preferred_element_type=F32)
             + jnp.dot(xn8[:, D // 2:], wq_v[1, :, cols], preferred_element_type=F32))
        for t in range(4):
            q_v[c * 4 + t] = q[:, t * DH:(t + 1) * DH]
    per_head(project, LAG + 24, 1)
    send(LAG + 24 + G, NR - LAG - 24 - G)

    def probs(g, hh):
        s = jax.lax.dot_general(q_v[g * G + hh].astype(BF16), kv_v[0, g, hh], _NT,
                                preferred_element_type=F32) * DH ** -0.5
        p = jnp.exp(s - jnp.max(s, axis=-1, keepdims=True))
        p_v[hh] = p
        l_v[hh] = jnp.broadcast_to(jnp.sum(p, axis=-1, keepdims=True), (8, DH))

    def attend(g, hh):
        o = jnp.dot(p_v[hh].astype(BF16), kv_v[1, g, hh], preferred_element_type=F32)
        o_v[g * G + hh] = o / l_v[hh]

    edges = [sum(VS[:c]) for c in range(len(VS) + 1)]

    def v_last(n, u):
        j = n - LAG + VS[0] - (NG - 1) * NR
        return kv(1, n - LAG + VS[0], u, s_v.at[sum(jnp.where(j >= e, 1, 0) for e in edges[1:-1])])

    def group(g, c):
        n0 = (g + 1) * NR
        send(n0, QK0)
        _wait_all(kv_v.at[0, g], s_kv.at[0, g % 2])
        per_head(lambda hh: probs(g, hh), n0 + QK0, 2)
        send(n0 + QK0 + 2 * G, LAG - QK0 - 2 * G)

        def rest(*pieces):
            send(n0 + LAG, NR - 2 * G - LAG, *pieces)
            _wait_all(kv_v.at[1, g], s_kv.at[1, g % 2])
            per_head(lambda hh: attend(g, hh), n0 + NR - 2 * G, 2, *pieces)
        pl.when(g < NG - 2)(rest)
        pl.when(g == NG - 2)(lambda: rest(v_last))
        return c
    jax.lax.fori_loop(0, NG - 1, group, 0)

    g = NG - 1
    n0 = NG * NR + VS[0]
    CH = DH // WR
    tail_edges = [sum(TAIL[:c]) for c in range(1, len(TAIL))]

    def wo_main(n, u):
        return wo(n - n0, u, s_wo.at[(n - n0) // CH])

    def wo_tail(n, u):
        m = n - n0 - (NB - TA)
        return wo(NB + m, u, s_t.at[sum(jnp.where(4 * m + u >= e, 1, 0) for e in tail_edges)])

    def attend_slice(c):
        rows = pl.ds(edges[c] * PR, VS[c] * PR)
        _wait_all(kv_v.at[1, g, :, rows], s_v.at[c])

        def work(hh):
            o = jnp.dot(p_v[hh, :, rows].astype(BF16), kv_v[1, g, hh, rows], preferred_element_type=F32)
            if c > 0:
                o = o + o_v[g * G + hh]
            o_v[g * G + hh] = o / l_v[hh] if c == len(VS) - 1 else o
        return work

    def project_out(acc, r0, r1, heads):
        for h in heads:
            lo, hi = max(r0, h % 4 * DH), min(r1, (h % 4 + 1) * DH)
            if lo < hi:
                acc = acc + jnp.dot(o_v[h].astype(BF16)[:, lo % DH:lo % DH + hi - lo],
                                    wo_v[h // 16, h // 4 % 4, pl.ds(lo, hi - lo), :], preferred_element_type=F32)
        return acc

    def columns(heads):
        for h in heads:
            if h % 4 == 3:
                o = o_v[h].astype(BF16).astype(F32)
                c_v[h // 4] = jnp.broadcast_to(o[0:1], (DH, DH)).T

    def wait_wo(c):
        _wait_all(wo_v.at[:, :, pl.ds(c * DH, DH), :], s_wo.at[c])

    assert (NB - TA) % G == 0 and TA % G == 0 and sum(TAIL) == 4 * TA and sum(VS) == NR
    send(NG * NR, VS[0], v_last, lambda n, u: kv(1, n - NR, u, s_v.at[0]))
    _wait_all(kv_v.at[0, g], s_kv.at[0, g % 2])
    per_head(lambda hh: probs(g, hh), n0, (NB - TA) // G, v_last, wo_main)
    slice0, slice1 = attend_slice(0), attend_slice(1)
    per_head(lambda hh: (slice0(hh), slice1(hh)), n0 + NB - TA, TA // G, wo_tail, wo_main)

    early, last = range(NH - G), range(NH - G, NH)
    acc = jnp.zeros((8, D), F32)
    columns(early)
    for c in range(2, len(VS)):
        if c - 2 < NB // CH - 1:
            wait_wo(c - 2)
            acc = project_out(acc, (c - 2) * DH, (c - 1) * DH, early)
        work = attend_slice(c)
        for hh in range(G):
            work(hh)
    columns(last)
    acc = project_out(acc, 0, NB * WR - DH, last)
    wait_wo(NB // CH - 1)
    acc = project_out(acc, NB * WR - DH, NB * WR, range(NH))

    part = jnp.zeros((8, D), F32)
    row = jax.lax.broadcasted_iota(jnp.int32, (8, D), 0)
    i0 = 0
    for c, n in enumerate(TAIL):
        r0 = (NB + i0 // 4) * WR
        blocks = slice(None) if n % 4 == 0 else pl.ds(i0 % 4, n)
        _wait_all(wo_v.at[:, blocks, pl.ds(r0, pl.cdiv(n, 4) * WR), :], s_t.at[c])
        if c == 0:
            acc = project_out(acc, r0, r0 + n // 4 * WR, range(NH))
        else:
            for i in range(i0, i0 + n):
                for k in range(2):
                    coef = c_v[4 * k + i % 4, pl.ds(i // 4 * WR, WR), :]
                    t = (wo_v[k, i % 4, pl.ds((NB + i // 4) * WR, WR), :].astype(F32)
                         * jnp.concatenate([coef] * (D // DH), axis=1))
                    part = part + (t[:8] + t[8:])
        if c == 2:
            part = part + jnp.where(row == 0, acc, 0.0)
        i0 += n
    s_out = jnp.sum(part, axis=0, keepdims=True)

    res = x8 + jnp.broadcast_to(s_out, (8, D)) * gate
    out_ref[0] = res.astype(out_ref.dtype)[0:1]


@jax.jit
def pallas_recurrent_scan__sliding_block_cached__moe_arch_mod__decode_kernel(
    A_x: jax.Array,
    A_k_cache: jax.Array,
    A_v_cache: jax.Array,
    A_wq: jax.Array,
    A_wo: jax.Array,
    B_x: jax.Array,
    B_w_r: jax.Array,
    B_w_gate: jax.Array,
    B_w_up: jax.Array,
    B_w_down: jax.Array,
):
    del B_x
    hbm = pl.BlockSpec(memory_space=pltpu.HBM)
    dma = pltpu.SemaphoreType.DMA
    halves = (2, F // 2, D)
    return pl.pallas_call(
        _kernel,
        out_shape=jax.ShapeDtypeStruct((1, 1, D), BF16),
        in_specs=[hbm] * 9,
        out_specs=pl.BlockSpec(memory_space=pltpu.VMEM),
        scratch_shapes=[
            pltpu.VMEM((1, 1, D), BF16),
            pltpu.VMEM((D,), BF16),
            pltpu.VMEM((2, D // 2, NH * DH), BF16),
            pltpu.VMEM((2, NG, G, W, DH), BF16),
            pltpu.VMEM((2, 4, OB, D), BF16),
            pltpu.VMEM((3,) + halves, BF16),
            pltpu.VMEM((NH, 8, DH), F32),
            pltpu.VMEM((NH, 8, DH), F32),
            pltpu.VMEM((G, 8, W), F32),
            pltpu.VMEM((G, 8, DH), F32),
            pltpu.VMEM((8, DH, DH), F32),
            dma((2,)), dma((2,)), dma((2, 2)), dma((len(VS),)), dma((NB * WR // DH,)), dma((len(TAIL),)),
        ],
        compiler_params=pltpu.CompilerParams(
            vmem_limit_bytes=100 * 1024 * 1024,
            disable_semaphore_checks=True,
        ),
    )(A_x, A_k_cache, A_v_cache, A_wq.reshape(2, D // 2, NH * DH), A_wo.reshape(2, 4, OB, D), B_w_r,
      B_w_gate.T.reshape(halves), B_w_up.T.reshape(halves), B_w_down.reshape(halves))
```
